```python
import jax
import jax.numpy as jnp

def _softmax(x, axis=-1):
    return jax.nn.softmax(x, axis=axis)
def _gelu(x):
    return jax.nn.gelu(x, approximate=True)
def _silu(x):
    return jax.nn.silu(x)
def _sigmoid(x):
    return jax.nn.sigmoid(x)
def _layernorm(x, axis=-1, eps=1e-5):
    m = jnp.mean(x, axis=axis, keepdims=True)
    v = jnp.var(x, axis=axis, keepdims=True)
    return (x - m) / jnp.sqrt(v + eps)
def _scatter_add(tgt, idx, src, axis=0):
    return tgt.at[idx].add(src)
def _segment_sum(src, seg, n):
    return jax.ops.segment_sum(src, seg, n)
class _Rng:
    def __init__(self, key):
        self._k = key
    def _next(self):
        self._k, sub = jax.random.split(self._k)
        return sub
    def normal(self, shape):
        return jax.random.normal(self._next(), shape, dtype=jnp.bfloat16)
    def randint(self, lo, hi, shape):
        return jax.random.randint(self._next(), shape, lo, hi, dtype=jnp.int32)
    def uniform(self, shape, lo=0.0, hi=1.0):
        return jax.random.uniform(self._next(), shape, jnp.bfloat16, lo, hi)
    def permutation(self, n):
        return jax.random.permutation(self._next(), n)


kernel_name = 'gated_mix__sliding_local_dilated__compressed_kv_cla__prompt'

def setup_inputs():
    _rng = _Rng(jax.random.key(int.from_bytes(__import__("os").urandom(4), "little")))
    _w = (lambda a: (lambda t: t.astype(jnp.bfloat16) if jnp.issubdtype(t.dtype, jnp.floating) else t)(jnp.asarray(a)))
    def _A_setup():
        B, S, D = 1, 2048, 576
        return {
            "x": _w((lambda *s: _rng.normal(s) * 0.05)(B, S, D)),
            "wqkv": _w((lambda *s: _rng.normal(s) * 0.05)(D, 3 * D)),
            "wo": _w((lambda *s: _rng.normal(s) * 0.05)(D, D)),
        }
    _A_in = _A_setup()

    def _B_setup():
        B, H, Sq, Sk, D, M = 1, 32, 2048, 2048, 128, 576
        Dc = 4 * D
        return {
            "x": _w((lambda *s: _rng.normal(s) * 0.05)(B, Sq, M)),
            "c_kv": _w((lambda *s: _rng.normal(s) * 0.05)(B, Sk, Dc)),
            "w_q": _w((lambda *s: _rng.normal(s) * 0.05)(M, H, D) * (M ** -0.5)),
            "w_uk": _w((lambda *s: _rng.normal(s) * 0.05)(Dc, H, D) * (Dc ** -0.5)),
            "w_uv": _w((lambda *s: _rng.normal(s) * 0.05)(Dc, H, D) * (Dc ** -0.5)),
            "w_o": _w((lambda *s: _rng.normal(s) * 0.05)(H, D, M) * ((H * D) ** -0.5)),
        }
    _B_in = _B_setup()

    return {
        "A_x": _A_in["x"],
        "A_wqkv": _A_in["wqkv"],
        "A_wo": _A_in["wo"],
        "B_x": _B_in["x"],
        "B_c_kv": _B_in["c_kv"],
        "B_w_q": _B_in["w_q"],
        "B_w_uk": _B_in["w_uk"],
        "B_w_uv": _B_in["w_uv"],
        "B_w_o": _B_in["w_o"],
        "gate_w": _w((lambda *s: _rng.normal(s) * 0.05)(576)),
    }

def reference(A_x, A_wqkv, A_wo, B_x, B_c_kv, B_w_q, B_w_uk, B_w_uv, B_w_o, gate_w):
    def _A_ref(x, wqkv, wo):
        B, S, D = x.shape
        H = 32; Dh = D // H
        W, dil = 8, 2
        qkv = (lambda x, *d: x.transpose(*d))((x @ wqkv).reshape(B, S, 3, H, Dh), 2, 0, 3, 1, 4)
        q, k, v = qkv[0], qkv[1], qkv[2]
        scale = Dh ** -0.5
        pos = jnp.arange(S)
        off = jnp.arange(W) * dil
        idx = pos[:, None] - off[None, :]
        mask = idx >= 0
        idx_c = jnp.where(mask, idx, 0).reshape(-1)
        kg = k[:, :, idx_c, :].reshape(B, H, S, W, Dh)
        vg = v[:, :, idx_c, :].reshape(B, H, S, W, Dh)
        logits = jnp.einsum("bhsd,bhswd->bhsw", q, kg) * scale
        logits = jnp.where(mask[None, None, :, :], logits, -1e9)
        attn = _softmax(logits, axis=-1)
        o = jnp.einsum("bhsw,bhswd->bhsd", attn, vg)
        return (lambda x, *d: x.transpose(*d))(o, 0, 2, 1, 3).reshape(B, S, D) @ wo

    def _B_ref(x, c_kv, w_q, w_uk, w_uv, w_o):
        B, Sq, M = x.shape[0], x.shape[1], x.shape[2]
        Sk = c_kv.shape[1]
        H, D = w_q.shape[1], w_q.shape[2]
        q = jnp.einsum("bqm,mhd->bhqd", x, w_q)
        k = jnp.einsum("bkc,chd->bhkd", c_kv, w_uk)
        v = jnp.einsum("bkc,chd->bhkd", c_kv, w_uv)
        scores = jnp.einsum("bhqd,bhkd->bhqk", q, k) * (D ** -0.5)
        off = Sk - Sq
        qi = jnp.arange(Sq)[:, None]
        kj = jnp.arange(Sk)[None, :]
        cmask = kj <= (qi + off)
        scores = jnp.where(cmask[None, None], scores, -1e9)
        p = _softmax(scores, axis=-1)
        ctx = jnp.einsum("bhqk,bhkd->bhqd", p, v)
        return jnp.einsum("bhqd,hdm->bqm", ctx, w_o)

    x = A_x
    g = _sigmoid((x * gate_w).sum(-1, keepdims=True))
    a = _A_ref(x, A_wqkv, A_wo)
    b = _B_ref(x, B_c_kv, B_w_q, B_w_uk, B_w_uv, B_w_o)
    return g * a + (1 - g) * b
```

```python
import jax
import jax.numpy as jnp
import numpy as np
from jax import lax
import jax.experimental.pallas as pl
import jax.experimental.pallas.tpu as pltpu

S = 2048
M = 576
H = 32
D = 128
DC = 512
DH = 18
W = 8
DIL = 2
HALO = 16
BQ = 256
ORDER = [1,3,5,7,6,4,2,0]
PM, PN = 512, 4
RB = 512
NF = S // RB
NP = H // 4
LOG2E = 1.4426950408889634
NT = (((1,), (1,)), ((), ()))
F32 = jnp.float32
BF16 = jnp.bfloat16


def _dot(a, b):
    return jnp.dot(a, b, preferred_element_type=F32)


def _heads(w_s, j):
    n = w_s.shape[0] // 16
    out = []
    for jj in (j, j + 1):
        e = w_s[pl.ds(jj, n, stride=16), :]
        o = w_s[pl.ds(jj + 8, n, stride=16), :]
        out.append(pltpu.bitcast((e & jnp.uint32(0xFFFF)) | (o << 16), BF16))
        out.append(pltpu.bitcast((e >> 16) | (o & jnp.uint32(0xFFFF0000)), BF16))
    return jnp.concatenate(out, axis=1)


def _kernel(xt_hbm, wqkv_hbm, wo_hbm, c_hbm, wq_hbm, wuk_hbm, wuv_hbm, wob_hbm, gw_ref,
            o_ref, sem, xt_ref, c_ref, wqkv_in, wo_in, tmp, wqkv_ref, wo_ref, wob_ref, wq_ref, wuk_ref, wuv_ref,
            x_ref, wq_s, wk_s, wv_s, wq4, wkv4, q_s, k_s, v_s, ctx_s, qa_s, ka_s, va_s):
    t = pl.program_id(0)
    late = [pltpu.make_async_copy(a, b, sem.at[n]) for n, (a, b) in enumerate(
        ((wqkv_hbm, wqkv_in), (wo_hbm, wo_in), (wob_hbm, wob_ref)))]
    half = [[pltpu.make_async_copy(a.at[:, pl.ds(16 * g, 16), :], b, sem.at[3 + n]) for n, (a, b) in enumerate(
        ((wq_hbm, wq_ref), (wuk_hbm, wuk_ref), (wuv_hbm, wuv_ref)))] for g in range(2)]

    @pl.when(t == 0)
    def _():
        cx = pltpu.make_async_copy(xt_hbm, xt_ref, sem.at[6])
        cc = pltpu.make_async_copy(c_hbm, c_ref, sem.at[7])
        for cp in [cx] + half[0] + [cc]:
            cp.start()
        cx.wait()
        x_ref[...] = xt_ref[...].T
        cc.wait()

    @pl.when(jnp.logical_and(t < NP, t % 4 == 0))
    def _():
        for cp, src, dst in zip(half[0], (wq_ref, wuk_ref, wuv_ref), (wq_s, wk_s, wv_s)):
            cp.wait()
            dst[...] = pltpu.bitcast(src[...], jnp.uint32).reshape(dst.shape)

    @pl.when(t == 1)
    def _():
        for cp in half[1] + late:
            cp.start()

    @pl.when(t == NP)
    def _():
        for cp in late:
            cp.wait()
        for r in (ka_s, va_s):
            r[0:HALO, :] = jnp.zeros((HALO, 640), F32)
        zero = jnp.zeros((64, D), F32)

        def regroup(base):
            return jnp.concatenate(
                [tmp[pl.ds(base + d, H, stride=DH), :] for d in range(DH)] + [zero], axis=0)

        for k0 in range(0, M, D):
            n = min(D, M - k0)
            blk = wqkv_in[k0:k0 + n, :].astype(F32)
            if n < D:
                blk = jnp.concatenate([blk, jnp.zeros((D - n, 3 * M), F32)], axis=0)
            tmp[...] = blk.T
            for part in range(3):
                wqkv_ref[part * 640:(part + 1) * 640, k0:k0 + n] = regroup(part * M)[:, :n].astype(BF16)
            blk = wo_in[:, k0:k0 + n].astype(F32)
            if n < D:
                blk = jnp.concatenate([blk, jnp.zeros((M, D - n), F32)], axis=1)
            tmp[0:M, :] = blk
            wo_ref[k0:k0 + n, :] = regroup(0).T[:n, :].astype(BF16)

    @pl.when(t < NP)
    def _():
        j = (t % 4) * 2
        wq4[...] = _heads(wq_s, j)
        wkv4[:, 0:4 * D] = _heads(wk_s, j)
        wkv4[:, 4 * D:] = _heads(wv_s, j)

        @pl.loop(0, S // PM)
        def _(i):
            rows = pl.ds(pl.multiple_of(i * PM, PM), PM)
            q = (_dot(x_ref[rows, :], wq4[...]) * (D ** -0.5 * LOG2E)).astype(BF16)
            kv = _dot(c_ref[rows, :], wkv4[...]).astype(BF16)
            for hh in range(4):
                q_s[hh, rows, :] = q[:, hh * D:(hh + 1) * D]
                k_s[hh, rows, :] = kv[:, hh * D:(hh + 1) * D]
                v_s[hh, rows, :] = kv[:, (4 + hh) * D:(5 + hh) * D]

        row = lax.broadcasted_iota(jnp.int32, (BQ, BQ), 0)
        col = lax.broadcasted_iota(jnp.int32, (BQ, BQ), 1)

        @pl.loop(0, 4)
        def _(h):
            HB = BQ // 2

            def scores(i):
                r0, n = i * BQ, (i + 1) * BQ
                full = lax.dot_general(q_s[h, r0:n, :], k_s[h, 0:n - HB, :], NT, preferred_element_type=F32)
                last = lax.dot_general(q_s[h, r0 + HB:n, :], k_s[h, n - HB:n, :], NT, preferred_element_type=F32)
                return full, last

            order = ORDER
            nxt = scores(order[0])
            for a, i in enumerate(order):
                r0, n = i * BQ, (i + 1) * BQ
                s, last = nxt
                if a + 1 < len(order):
                    nxt = scores(order[a + 1])
                sd = jnp.where(col[:, :HB] <= row[:, :HB], s[:, r0:], -1e9 * LOG2E)
                s = jnp.concatenate([s[:, :r0], sd], axis=1) if i > 0 else sd
                last = jnp.where(col[:HB, :HB] <= row[:HB, :HB], last, -1e9 * LOG2E)
                m = jnp.max(s, axis=1, keepdims=True)
                m = jnp.concatenate([m[:HB], jnp.maximum(m[HB:], jnp.max(last, axis=1, keepdims=True))], axis=0)
                p = jnp.exp2(s - m)
                pl_ = jnp.exp2(last - m[HB:])
                l = jnp.sum(p, axis=1, keepdims=True)
                o = _dot(p.astype(BF16), v_s[h, 0:n - HB, :])
                o2 = o[HB:] + _dot(pl_.astype(BF16), v_s[h, n - HB:n, :])
                l2 = l[HB:] + jnp.sum(pl_, axis=1, keepdims=True)
                ctx_s[t * 4 + h, r0:r0 + HB, :] = (o[:HB] / l[:HB]).astype(BF16)
                ctx_s[t * 4 + h, r0 + HB:n, :] = (o2 / l2).astype(BF16)

    @pl.when(t >= NP)
    def _():
        f = t - NP
        r0 = pl.multiple_of(f * RB, RB)
        x = x_ref[pl.ds(r0, RB), :]

        @pl.when(f > 0)
        def _():
            ka_s[0:HALO, :] = ka_s[RB:RB + HALO, :]
            va_s[0:HALO, :] = va_s[RB:RB + HALO, :]

        qkv = lax.dot_general(x, wqkv_ref[...], NT, preferred_element_type=F32)
        qa_s[...] = qkv[:, 0:640].astype(BF16).astype(F32)
        ka_s[pl.ds(HALO, RB), :] = qkv[:, 640:1280].astype(BF16).astype(F32)
        va_s[pl.ds(HALO, RB), :] = qkv[:, 1280:1920].astype(BF16).astype(F32)

        for r in (ka_s, va_s):
            r[0:HALO, :] = jnp.where(f == 0, jnp.broadcast_to(r[HALO:HALO + 1, :], (HALO, 640)), r[0:HALO, :])

        pos = r0 + lax.broadcasted_iota(jnp.int32, (RB, 128), 0)
        q = qa_s[...]
        ls = []
        for w in range(W):
            pr = q * ka_s[pl.ds(HALO - DIL * w, RB), :]
            a = pr[:, 0:128] + pr[:, 128:256] + pr[:, 256:384] + pr[:, 384:512] + pr[:, 512:640]
            a = a + pltpu.roll(a, 64, 1)
            a = a + pltpu.roll(a, 32, 1)
            ls.append(jnp.where(pos >= DIL * w, a * (DH ** -0.5), -1e9))
        m = ls[0]
        for w in range(1, W):
            m = jnp.maximum(m, ls[w])
        es = [jnp.exp(a - m) for a in ls]
        z = es[0]
        for w in range(1, W):
            z = z + es[w]
        o = None
        for w in range(W):
            p = es[w] / z
            pv = jnp.concatenate([p] * 5, axis=1) * va_s[pl.ds(HALO - DIL * w, RB), :]
            o = pv if o is None else o + pv
        a = lax.dot_general(wo_ref[...], o.astype(BF16), NT, preferred_element_type=F32)
        b = None
        for h in range(H):
            d = lax.dot_general(wob_ref[h], ctx_s[h, pl.ds(r0, RB), :], NT, preferred_element_type=F32)
            b = d if b is None else b + d
        g = _dot(jnp.broadcast_to(gw_ref[...].astype(F32).reshape(1, M), (16, M)).astype(BF16), xt_ref[:, pl.ds(r0, RB)])[0:1, :]
        g = jax.nn.sigmoid(g)
        o_ref[...] = (g * a + (1.0 - g) * b).astype(o_ref.dtype)


@jax.jit
def pallas_gated_mix__sliding_local_dilated__compressed_kv_cla__prompt_kernel(
    A_x, A_wqkv, A_wo, B_x, B_c_kv, B_w_q, B_w_uk, B_w_uv, B_w_o, gate_w,
):
    full = lambda shape: pl.BlockSpec(shape, lambda t: (0,) * len(shape), pipeline_mode=pl.Buffered(1))
    hbm = pl.BlockSpec(memory_space=pltpu.MemorySpace.HBM)
    out = pl.pallas_call(
        _kernel,
        grid=(NP + NF,),
        in_specs=[hbm, hbm, hbm, hbm, hbm, hbm, hbm, hbm, full((M,))],
        out_specs=pl.BlockSpec((M, RB), lambda t: (0, jnp.maximum(t - NP, 0))),
        out_shape=jax.ShapeDtypeStruct((M, S), A_x.dtype),
        scratch_shapes=[
            pltpu.SemaphoreType.DMA((8,)), pltpu.VMEM((M, S), BF16), pltpu.VMEM((S, DC), BF16),
            pltpu.VMEM((M, 3 * M), BF16), pltpu.VMEM((M, M), BF16), pltpu.VMEM((3 * M, D), F32),
            pltpu.VMEM((1920, M), BF16), pltpu.VMEM((M, 640), BF16), pltpu.VMEM((H, M, D), BF16),
            pltpu.VMEM((M, 16, D), BF16), pltpu.VMEM((DC, 16, D), BF16), pltpu.VMEM((DC, 16, D), BF16),
            pltpu.VMEM((S, M), BF16), pltpu.VMEM((M * 8, D), jnp.uint32),
            pltpu.VMEM((DC * 8, D), jnp.uint32), pltpu.VMEM((DC * 8, D), jnp.uint32),
            pltpu.VMEM((M, 4 * D), BF16), pltpu.VMEM((DC, 8 * D), BF16),
            pltpu.VMEM((4, S, D), BF16), pltpu.VMEM((4, S, D), BF16), pltpu.VMEM((4, S, D), BF16),
            pltpu.VMEM((H, S, D), BF16),
            pltpu.VMEM((RB, 640), F32), pltpu.VMEM((RB + HALO, 640), F32), pltpu.VMEM((RB + HALO, 640), F32),
        ],
        compiler_params=pltpu.CompilerParams(
            dimension_semantics=("arbitrary",), vmem_limit_bytes=110 * 1024 * 1024),
    )(A_x.reshape(S, M).T, A_wqkv, A_wo, B_c_kv.reshape(S, DC), B_w_q, B_w_uk, B_w_uv,
      B_w_o.transpose(0, 2, 1), gate_w)
    return out.T.reshape(1, S, M)
```
